```python
import os as _os
_os.environ.setdefault("JAX_PLATFORMS", "cpu")
import jax
import jax.numpy as jnp

def _softmax(x, axis=-1):
    return jax.nn.softmax(x, axis=axis)
def _gelu(x):
    return jax.nn.gelu(x, approximate=True)
def _silu(x):
    return jax.nn.silu(x)
def _sigmoid(x):
    return jax.nn.sigmoid(x)
def _layernorm(x, axis=-1, eps=1e-5):
    m = jnp.mean(x, axis=axis, keepdims=True)
    v = jnp.var(x, axis=axis, keepdims=True)
    return (x - m) / jnp.sqrt(v + eps)
def _scatter_add(tgt, idx, src, axis=0):
    return tgt.at[idx].add(src)
def _segment_sum(src, seg, n):
    return jax.ops.segment_sum(src, seg, n)
class _Rng:
    def __init__(self, key):
        self._k = key
    def _next(self):
        self._k, sub = jax.random.split(self._k)
        return sub
    def normal(self, shape):
        return jax.random.normal(self._next(), shape, dtype=jnp.bfloat16)
    def randint(self, lo, hi, shape):
        return jax.random.randint(self._next(), shape, lo, hi, dtype=jnp.int32)
    def uniform(self, shape, lo=0.0, hi=1.0):
        return jax.random.uniform(self._next(), shape, jnp.bfloat16, lo, hi)
    def permutation(self, n):
        return jax.random.permutation(self._next(), n)


kernel_name = 'gated_mix__grouped_kv_mqa__glu_gated_reglu__prompt'

def setup_inputs():
    _rng = _Rng(jax.random.key(int.from_bytes(__import__("os").urandom(4), "little")))
    _w = (lambda a: (lambda t: t.astype(jnp.bfloat16) if jnp.issubdtype(t.dtype, jnp.floating) else t)(jnp.asarray(a)))
    def _A_setup():
        B, S, D, H = 1, 2048, 1024, 32
        Dh = D // H
        return {
            "x": _w((lambda *s: _rng.normal(s) * 0.05)(B, S, D)),
            "wq": _w((lambda *s: _rng.normal(s) * 0.2)(D, H * Dh)),
            "wk": _w((lambda *s: _rng.normal(s) * 0.2)(D, Dh)),
            "wv": _w((lambda *s: _rng.normal(s) * 0.05)(D, Dh)),
            "wo": _w((lambda *s: _rng.normal(s) * 0.05)(H * Dh, D)),
        }
    _A_in = _A_setup()

    def _B_setup():
        B, S, D, F = 1, 2048, 1024, 3584
        return {
            "x": _w((lambda *s: _rng.normal(s) * 0.05)(B, S, D)),
            "W_gate": _w((lambda *s: _rng.normal(s) * 0.8)(D, F) * (2.0 / D) ** 0.5),
            "W_up": _w((lambda *s: _rng.normal(s) * 0.8)(D, F) * (2.0 / D) ** 0.5),
            "W_down": _w((lambda *s: _rng.normal(s) * 0.8)(F, D) * (1.0 / F) ** 0.5),
        }
    _B_in = _B_setup()

    return {
        "A_x": _A_in["x"],
        "A_wq": _A_in["wq"],
        "A_wk": _A_in["wk"],
        "A_wv": _A_in["wv"],
        "A_wo": _A_in["wo"],
        "B_x": _B_in["x"],
        "B_W_gate": _B_in["W_gate"],
        "B_W_up": _B_in["W_up"],
        "B_W_down": _B_in["W_down"],
        "gate_w": _w((lambda *s: _rng.normal(s) * 0.05)(1024) * 16.0),
    }

def reference(A_x, A_wq, A_wk, A_wv, A_wo, B_x, B_W_gate, B_W_up, B_W_down, gate_w):
    def _A_ref(x, wq, wk, wv, wo):
        B, S, D = x.shape
        H = 32
        Dh = D // H
        q = (lambda x, *d: x.transpose(*d))((x @ wq).reshape(B, S, H, Dh), 0, 2, 1, 3)
        k = x @ wk
        v = x @ wv
        scores = jnp.einsum("bhqd,bkd->bhqk", q, k) * (Dh ** -0.5)
        p = _softmax(scores, axis=-1)
        o = jnp.einsum("bhqk,bkd->bhqd", p, v)
        return (lambda x, *d: x.transpose(*d))(o, 0, 2, 1, 3).reshape(B, S, H * Dh) @ wo

    def _B_ref(x, W_gate, W_up, W_down):
        gate = jnp.einsum("bsd,df->bsf", x, W_gate)
        up = jnp.einsum("bsd,df->bsf", x, W_up)
        gate = gate * (lambda x, dt: x.astype(dt))(gate > 0, gate.dtype)
        h = gate * up
        return jnp.einsum("bsf,fd->bsd", h, W_down)

    x = A_x
    g = _sigmoid((x * gate_w).sum(-1, keepdims=True))
    a = _A_ref(x, A_wq, A_wk, A_wv, A_wo)
    b = _B_ref(x, B_W_gate, B_W_up, B_W_down)
    return g * a + (1 - g) * b
```

```python
import functools
import math

import jax
import jax.numpy as jnp
from jax import lax
from jax.experimental import pallas as pl
from jax.experimental.pallas import tpu as pltpu

S = 2048
D = 1024
H = 32
DH = 32
F = 3584
TQ = 256
NB = S // TQ
NSUB = 4
HPS = H // NSUB
FS = F // NSUB
QS = D // NSUB
KC = 128
NKC = S // KC
XC = 256
NXC = S // XC

_NT = (((1,), (1,)), ((), ()))
_F32 = jnp.float32
_BF16 = jnp.bfloat16
_QSCALE = (DH ** -0.5) * math.log2(math.e)


def _dot(a, b):
    return jnp.dot(a, b, preferred_element_type=_F32)


def _pack(a):
    return pltpu.bitcast(a, jnp.uint32)


def _unpack(a):
    return pltpu.bitcast(a, _BF16)


def make_kernel(LAG=5, EVERY=5, START=2):
    def kernel(x_hbm, wq_hbm, wk_hbm, wv_hbm, wo_hbm, wg_hbm, wu_hbm, wd_hbm, gw_hbm,
               out_ref,
               x_v, wq_v, wk_v, wv_v, wo_v, wg_v, wu_v, wd_v, gw_v,
               kp_v, vt_v, g_v, q_v, acc_v, sems):
        b = pl.program_id(0)
        sub = pl.program_id(1)

        def cp_x(c):
            return pltpu.make_async_copy(x_hbm.at[pl.ds(c * XC, XC), :], x_v.at[pl.ds(c * XC, XC), :], sems.at[c])
        base = NXC
        cp_wk = lambda: pltpu.make_async_copy(wk_hbm, wk_v, sems.at[base])
        cp_wv = lambda: pltpu.make_async_copy(wv_hbm, wv_v, sems.at[base + 1])
        cp_gw = lambda: pltpu.make_async_copy(gw_hbm, gw_v, sems.at[base + 2])
        base2 = base + 3
        cp_wq = lambda i: pltpu.make_async_copy(wq_hbm.at[:, pl.ds(i * QS, QS)], wq_v.at[i], sems.at[base2 + i])
        cp_wo = lambda i: pltpu.make_async_copy(wo_hbm.at[pl.ds(i * QS, QS), :], wo_v.at[i], sems.at[base2 + 4 + i])
        cp_wg = lambda i: pltpu.make_async_copy(wg_hbm.at[:, pl.ds(i * FS, FS)], wg_v.at[i], sems.at[base2 + 8 + i])
        cp_wu = lambda i: pltpu.make_async_copy(wu_hbm.at[:, pl.ds(i * FS, FS)], wu_v.at[i], sems.at[base2 + 12 + i])
        cp_wd = lambda i: pltpu.make_async_copy(wd_hbm.at[pl.ds(i * FS, FS), :], wd_v.at[i], sems.at[base2 + 16 + i])

        def qproj(xrows, wslot, g):
            q = _dot(xrows, wq_v[wslot, :, pl.ds(g * 128, 128)]) * _QSCALE
            q_v[g] = _pack(q.astype(_BF16))

        @pl.when(jnp.logical_and(b == 0, sub == 0))
        def _prologue():
            cp_wk().start(); cp_wv().start(); cp_gw().start()
            for c in range(NXC):
                cp_x(c).start()
            cp_wq(0).start()
            for i in range(NSUB):
                cp_wg(i).start(); cp_wu(i).start()
                if i + 1 < NSUB:
                    cp_wq(i + 1).start()
                cp_wd(i).start(); cp_wo(i).start()
            cp_wk().wait(); cp_wv().wait(); cp_gw().wait()
            wkv = jnp.concatenate(
                [wk_v[...], wv_v[...], jnp.zeros((D, 64), _BF16)], axis=1)
            gw = gw_v[...].astype(_F32)
            lane = lax.broadcasted_iota(jnp.int32, (XC, 128), 1)
            for c in range(NXC):
                cp_x(c).wait()
                xc = x_v[pl.ds(c * XC, XC), :]
                r = _dot(xc, wkv)
                k0 = jnp.where(lane < DH, r, 0.0)
                for j in range(4):
                    kj = k0 if j == 0 else pltpu.roll(k0, DH * j, 1)
                    kp_v[j, pl.ds(c * XC // 2, XC // 2), :] = _pack(kj.astype(_BF16))
                rt = r.T
                vt_v[:, pl.ds(c * XC, XC)] = _pack(rt[DH:2 * DH, :].astype(_BF16))
                logit = jnp.sum(xc.astype(_F32) * gw, axis=1, keepdims=True)
                g_v[pl.ds(c * XC, XC), :] = jnp.broadcast_to(jax.nn.sigmoid(logit), (XC, 128))
            cp_wq(0).wait()
            x0 = x_v[pl.ds(0, TQ), :]
            qproj(x0, 0, 0)
            qproj(x0, 0, 1)

        @pl.when(b == 0)
        def _wait_weights():
            for i in range(NSUB):
                @pl.when(sub == i)
                def _():
                    cp_wg(i).wait(); cp_wu(i).wait(); cp_wd(i).wait(); cp_wo(i).wait()
                    if i + 1 < NSUB:
                        cp_wq(i + 1).wait()

        row0 = pl.multiple_of(b * TQ, TQ)
        nsub = (sub + 1) % NSUB
        nb = jnp.minimum(b + (sub + 1) // NSUB, NB - 1)
        nrow0 = pl.multiple_of(nb * TQ, TQ)
        xb = lambda: x_v[pl.ds(row0, TQ), :]
        gb = lambda: g_v[pl.ds(row0, TQ), :]

        svals = {}
        st = {}
        ot = {}

        def qk(u, c):
            kk = _unpack(kp_v[u % 4, pl.ds(c * KC // 2, KC // 2), :])
            svals[(u, c)] = lax.dot_general(kk, _unpack(q_v[u // 4]), _NT, preferred_element_type=_F32)

        def proc(u, c):
            s = svals.pop((u, c))
            mc = jnp.max(jnp.max(s.reshape(KC // 8, 8, TQ), axis=0), axis=0, keepdims=True)
            if c == 0:
                m = mc
            else:
                m0, l0, o0 = st[u]
                m = jnp.maximum(m0, mc)
                alpha = jnp.exp2(m0 - m)
            p = jnp.exp2(s - m)
            l = jnp.sum(p.reshape(KC // 8, 8, TQ), axis=0)
            o = _dot(_unpack(vt_v[:, pl.ds(c * KC, KC)]), p.astype(_BF16))
            if c > 0:
                l = l0 * alpha + l
                o = o0 * alpha + o
            st[u] = (m, l, o)
            if c == NKC - 1:
                lt = jnp.sum(l, axis=0, keepdims=True)
                ot[u] = o * (1.0 / lt)

        NF = FS // 128
        gate = {}
        hs = {}
        og = {}

        def p_gate(f):
            gate[f] = jnp.maximum(_dot(xb(), wg_v[sub, :, pl.ds(f * 128, 128)]), 0.0)

        def p_up(f):
            up = _dot(xb(), wu_v[sub, :, pl.ds(f * 128, 128)])
            hs[f] = (gate.pop(f) * up).astype(_BF16)

        def get_o(g):
            if g not in og:
                o4 = jnp.concatenate([ot[4 * g + j] for j in range(4)], axis=0)
                og[g] = o4.T.astype(_BF16)
            return og[g]

        def p_down(n):
            h = jnp.concatenate([hs[f] for f in range(NF)], axis=1)
            cols = pl.ds(n * 128, 128)
            g = gb()
            bb = _dot(h, wd_v[sub, :, cols])
            aa = _dot(get_o(0), wo_v[sub, pl.ds(0, 128), cols])
            prev = jnp.where(sub == 0, 0.0, acc_v[:, cols])
            acc_v[:, cols] = prev + (1.0 - g) * bb + g * aa

        def p_ofin():
            g = gb()
            o1 = get_o(1)
            for n in range(D // 256):
                cols = pl.ds(n * 256, 256)
                aa = _dot(o1, wo_v[sub, pl.ds(128, 128), cols])
                tot = acc_v[:, cols] + jnp.concatenate([g, g], axis=1) * aa
                acc_v[:, cols] = tot
                out_ref[:, cols] = tot.astype(_BF16)

        def p_q(g):
            qproj(x_v[pl.ds(nrow0, TQ), :], nsub, g)

        steps = [(u, c) for u in range(HPS) for c in range(NKC)]
        n = len(steps)
        early = []
        for f in range(NF):
            early += [functools.partial(p_gate, f), functools.partial(p_up, f)]
        late = [functools.partial(p_q, 0)] + [functools.partial(p_down, k) for k in range(D // 128)]
        sched = {}
        pos = START
        for pc in early:
            sched.setdefault(pos, []).append(pc)
            pos += EVERY
        pos = max(pos, 4 * NKC + LAG + 4)
        nl = len(late) - 2
        for pc in late[:nl]:
            sched.setdefault(min(pos, n - 1), []).append(pc)
            pos += EVERY
        sched.setdefault(n, []).append(functools.partial(p_q, 1))
        sched.setdefault(n + LAG - 1, []).extend(late[nl:])
        for i in range(n + LAG):
            if i < n:
                qk(*steps[i])
            if i >= LAG:
                proc(*steps[i - LAG])
            for pc in sched.get(i, []):
                pc()
        p_ofin()

    return kernel


def _build(**kw):
    nsem = NXC + 3 + 20
    any_spec = pl.BlockSpec(memory_space=pl.ANY)

    @jax.jit
    def fn(A_x, A_wq, A_wk, A_wv, A_wo, B_x, B_W_gate, B_W_up, B_W_down, gate_w):
        x = A_x.reshape(S, D)
        gw = gate_w.reshape(1, D)
        out = pl.pallas_call(
            make_kernel(**kw),
            grid=(NB, NSUB),
            in_specs=[any_spec] * 9,
            out_specs=pl.BlockSpec((TQ, D), lambda b, s: (b, 0)),
            out_shape=jax.ShapeDtypeStruct((S, D), _BF16),
            scratch_shapes=[
                pltpu.VMEM((S, D), _BF16),
                pltpu.VMEM((NSUB, D, QS), _BF16),
                pltpu.VMEM((D, DH), _BF16),
                pltpu.VMEM((D, DH), _BF16),
                pltpu.VMEM((NSUB, QS, D), _BF16),
                pltpu.VMEM((NSUB, D, FS), _BF16),
                pltpu.VMEM((NSUB, D, FS), _BF16),
                pltpu.VMEM((NSUB, FS, D), _BF16),
                pltpu.VMEM((1, D), _BF16),
                pltpu.VMEM((4, S // 2, 128), jnp.uint32),
                pltpu.VMEM((DH // 2, S), jnp.uint32),
                pltpu.VMEM((S, 128), _F32),
                pltpu.VMEM((2, TQ // 2, 128), jnp.uint32),
                pltpu.VMEM((TQ, D), _F32),
                pltpu.SemaphoreType.DMA((nsem,)),
            ],
            compiler_params=pltpu.CompilerParams(
                dimension_semantics=("arbitrary", "arbitrary"),
                vmem_limit_bytes=100 * 1024 * 1024),
            name="gmix",
        )(x, A_wq, A_wk, A_wv, A_wo, B_W_gate, B_W_up, B_W_down, gw)
        return out.reshape(1, S, D)
    return fn


pallas_gated_mix__grouped_kv_mqa__glu_gated_reglu__prompt_kernel = _build()
```

```python
import functools
import math

import jax
import jax.numpy as jnp
from jax import lax
from jax.experimental import pallas as pl
from jax.experimental.pallas import tpu as pltpu

S = 2048
D = 1024
H = 32
DH = 32
F = 3584
TQ = 256
NB = S // TQ
XC = 256
NXC = S // XC
NSUB = 4
HPS = H // NSUB
FS = F // NSUB
QS = D // NSUB
NG = QS // 128
NF = FS // 128
KC = 128
NKC = S // KC
NPAIR = NB // 2
NSTEP = NSUB * NPAIR
KG = 512
CPG = KG // KC

_NT = (((1,), (1,)), ((), ()))
_F32 = jnp.float32
_BF16 = jnp.bfloat16
_QSCALE = (DH ** -0.5) * math.log2(math.e)


def _dot(a, b):
    return jnp.dot(a, b, preferred_element_type=_F32)


def _pack(a):
    return pltpu.bitcast(a, jnp.uint32)


def _unpack(a):
    return pltpu.bitcast(a, _BF16)


def make_kernel(LAG=4, START=0, END=0, QOFF=0, LAG0=6, OSPLIT=8, ORD=0, PROF=0, SKIP1=0, NA=10, QM=2, EV=2, QPRE=0, QPRE0=0, QZ=16, QZG=0, QZD=16, KV0=-61, KV1=0, DG=9, DSP=4, ORD0=2, PLOOP=1, SKIPU=0):
    P = functools.partial
    OC = D // OSPLIT

    def kernel(x_hbm, wq_hbm, wkt_hbm, wvt_hbm, wo_hbm, wg_hbm, wu_hbm, wd_hbm, gw_hbm,
               out_hbm,
               x_v, wq_v, wkv_v, gw_v, wgu_v, wdo_v,
               k_v, vt_v, lg_v, g_v, q_v, acc_v, out_v, st_v, z_s, sems):
        cp = pltpu.make_async_copy
        cp_x = lambda c: cp(x_hbm.at[pl.ds(c * XC, XC), :], x_v.at[pl.ds(c * XC, XC), :], sems.at[c])
        s0 = NXC
        cp_wk = lambda: cp(wkt_hbm, wkv_v.at[pl.ds(0, DH), :], sems.at[s0])
        cp_wv = lambda: cp(wvt_hbm, wkv_v.at[pl.ds(DH, DH), :], sems.at[s0 + 1])
        cp_gw = lambda: cp(gw_hbm, gw_v, sems.at[s0 + 2])
        s1 = s0 + 3
        sx = lambda i: 0 if i == 0 else 3
        cp_wq = lambda i: cp(wq_hbm.at[:, pl.ds(i * QS, QS)], wq_v.at[i], sems.at[s1 + sx(i)])
        cp_wg = lambda i: cp(wg_hbm.at[:, pl.ds(i * FS, FS)], wgu_v.at[i, 0], sems.at[s1 + 1 + sx(i)])
        cp_wu = lambda i: cp(wu_hbm.at[:, pl.ds(i * FS, FS)], wgu_v.at[i, 1], sems.at[s1 + 1 + sx(i)])
        cp_wd = lambda i: cp(wd_hbm.at[pl.ds(i * FS, FS), :], wdo_v.at[i, pl.ds(0, FS), :], sems.at[s1 + 2 + sx(i)])
        cp_wo = lambda i: cp(wo_hbm.at[pl.ds(i * QS, QS), :], wdo_v.at[i, pl.ds(FS, QS), :], sems.at[s1 + 2 + sx(i)])
        s_out = s1 + 6

        def wait_view(view, k):
            cp(view, view, sems.at[k]).wait()

        def cp_out(rows, m, j):
            return cp(out_v.at[pl.ds(rows, m), pl.ds(j * OC, OC)],
                      out_hbm.at[pl.ds(rows, m), pl.ds(j * OC, OC)], sems.at[s_out])

        def kv_chunk(c):
            r0 = c * XC
            h0 = c * (XC // 2)
            if not isinstance(c, int):
                r0 = pl.multiple_of(r0, XC)
                h0 = pl.multiple_of(h0, XC // 2)
            xc = x_v[pl.ds(r0, XC), :]
            rt = lax.dot_general(wkv_v[...], xc, _NT, preferred_element_type=_F32)
            k_v[pl.ds(h0, XC // 2), :] = _pack(rt[0:DH, :].T.astype(_BF16))
            vt_v[c] = _pack(rt[DH:2 * DH, :].astype(_BF16))
            lg_v[c] = rt[2 * DH:2 * DH + 8, :]

        def g_fill(c):
            sg = jax.nn.sigmoid(lg_v[c])
            g_v[pl.ds(pl.multiple_of(c * XC, XC), XC), :] = jnp.concatenate([sg] * 16, axis=0).T

        def q_proj(slot, rows, blk, g, nb=1):
            r = _dot(x_v[pl.ds(rows, nb * TQ), :], wq_v[slot, :, pl.ds(g * 128, 128)])
            for k in range(nb):
                q_v[blk + k, g] = _pack((r[k * TQ:(k + 1) * TQ] * _QSCALE).T.astype(_BF16))

        class Attn:
            def __init__(self, kbase=0, preload=0, qslot=lambda blk: blk, qpre=(), qz=0):
                self.qz = qz
                self.qslot = qslot
                self.z = {}
                self.qc = {key: self.load_q(key) for key in qpre}
                self.s = {}
                self.st = {}
                self.kbase = kbase
                self.kc = {c: self.load_k(c) for c in range(preload)}
                self.vc = {c: self.load_v(c) for c in range(preload)}

            def load_k(self, c):
                h0 = self.kbase // 2 + c * (KC // 2)
                if not isinstance(h0, int):
                    h0 = pl.multiple_of(h0, KC // 2)
                return _unpack(k_v[pl.ds(h0, KC // 2), :])

            def load_v(self, c):
                vi = self.kbase // XC + (c * KC) // XC
                return _unpack(vt_v[vi, :, pl.ds((c * KC) % XC, KC)])

            def load_q(self, key, c=None):
                blk, u = key
                g = u // 4
                if self.qz and c is not None:
                    if c % self.qz not in self.z:
                        self.z[c % self.qz] = z_s[c % self.qz]
                    g = g + self.z[c % self.qz]
                return _unpack(q_v[self.qslot(blk), g, pl.ds((u % 4) * 16, 16), :])

            def qk(self, key, c):
                kk = self.kc[c] if c in self.kc else self.load_k(c)
                qt = self.qc[key] if key in self.qc else self.load_q(key, c)
                self.s[(key, c)] = _dot(kk, qt)

            def proc(self, key, c):
                s = self.s.pop((key, c))
                mc = jnp.max(jnp.max(s.reshape(KC // 8, 8, TQ), axis=0), axis=0, keepdims=True)
                prev = self.st.get(key)
                if prev is None:
                    m = mc
                else:
                    m0, l0, o0 = prev
                    m = jnp.maximum(m0, mc)
                    alpha = jnp.exp2(m0 - m)
                p = jnp.exp2(s - m)
                l = jnp.sum(p.reshape(KC // 8, 8, TQ), axis=0)
                vt = self.vc[c] if c in self.vc else self.load_v(c)
                o = _dot(vt, p.astype(_BF16))
                if prev is not None:
                    l = l0 * alpha + l
                    o = o0 * alpha + o
                self.st[key] = (m, l, o)

            def final(self, key):
                _, l, o = self.st[key]
                return o * (1.0 / jnp.sum(l, axis=0, keepdims=True))

        class Dense:
            def __init__(self, sub, row0, get_ot, first, nb=1):
                self.sub, self.row0, self.get_ot, self.first = sub, row0, get_ot, first
                self.nb, self.m = nb, nb * TQ
                self.part, self.hs, self.og, self.g = {}, {}, {}, None

            def gb(self):
                if self.g is None:
                    self.g = g_v[pl.ds(self.row0, self.m), :]
                return self.g

            def gate(self, f):
                r = _dot(x_v[pl.ds(self.row0, self.m), :], wgu_v[self.sub, 0, :, pl.ds(f * 128, 128)])
                self.part[f] = jnp.maximum(r, 0.0) * (1.0 - self.gb())

            def up(self, f):
                r = _dot(x_v[pl.ds(self.row0, self.m), :], wgu_v[self.sub, 1, :, pl.ds(f * 128, 128)])
                self.hs[f] = (self.part.pop(f) * r).astype(_BF16)

            def gu(self):
                return [P(fn, f) for f in range(NF) for fn in (self.gate, self.up)]

            def get_o(self, g):
                if g not in self.og:
                    o4 = [jnp.concatenate([self.get_ot(k, 4 * g + j) for j in range(4)], axis=0).T
                          for k in range(self.nb)]
                    self.og[g] = (jnp.concatenate(o4, axis=0) * self.gb()).astype(_BF16)
                return self.og[g]

            def down(self, n):
                cols = pl.ds(n * 128, 128)
                rows = pl.ds(self.row0, self.m)
                lhs = [self.hs[i] for i in range(NF)] + [self.get_o(i) for i in range(NG)]
                tot = _dot(jnp.concatenate(lhs, axis=1), wdo_v[self.sub, :, cols])
                if self.first:
                    acc_v[rows, cols] = tot
                else:
                    tot = jnp.where(self.sub == 0, 0.0, acc_v[rows, cols]) + tot
                    acc_v[rows, cols] = tot
                    out_v[rows, cols] = tot.astype(_BF16)
                    if ((n + 1) * 128) % OC == 0:
                        @pl.when(self.sub == NSUB - 1)
                        def _():
                            cp_out(self.row0, self.m, (n * 128) // OC).start()

            def downs(self):
                return [P(self.down, n) for n in range(D // 128)]

        def run(att, steps, lag, sched, order="qpd", pre=None, post=None):
            n = len(steps)
            for i in range(n + lag):
                acts = {
                    "q": (lambda: att.qk(*steps[i])) if i < n else None,
                    "p": (lambda: att.proc(*steps[i - lag])) if i >= lag else None,
                    "d": lambda: [fn() for fn in sched.get(i, [])],
                }
                if i >= lag and pre is not None:
                    pre(*steps[i - lag])
                for key in order:
                    if acts[key] is not None:
                        acts[key]()
                if i >= lag and post is not None:
                    post(*steps[i - lag])

        units = [(blk, u) for blk in range(2) for u in range(HPS)]

        def uniform(sub, row0, nsub, nrow0):
            att = Attn(qpre=units if QPRE == 1 else (), qz=QZ)
            steps = [(key, c) for key in units for c in range(NKC)]
            n = len(steps)
            sched = {}
            if QPRE > 1:
                def pf(key):
                    att.qc[key] = att.load_q(key)
                for k, key in enumerate(units[1:]):
                    sched.setdefault((k + 1) * NKC - QPRE, []).append(P(pf, key))
            dn = Dense(sub, row0, lambda k, u: att.final((k, u)), False, 2)
            gu = dn.gu()
            if QM == 2:
                qn = [P(q_proj, nsub, nrow0, 0, g, 2) for g in range(NG)]
                mid = []
            else:
                qn = [P(q_proj, nsub, nrow0 + TQ, 1, g) for g in range(NG)]
                mid = [P(q_proj, nsub, nrow0, 0, g) for g in range(NG)]
            rounds = gu[:NA] + mid + gu[NA:]
            for k, fn in enumerate(rounds):
                sched.setdefault(START + EV * ((k * ((n - START - END) // EV)) // len(rounds)), []).append(fn)
            sched.setdefault(n - 1 + QOFF, []).append(qn[0])
            run(att, steps, LAG, sched, ["qpd", "pqd", "qdp"][ORD])
            for fn in qn[1:] + dn.downs():
                fn()

        cp_x(0).start()
        cp_wk().start(); cp_wv().start(); cp_gw().start()
        cp_wq(0).start()
        for c in range(1, NXC):
            cp_x(c).start()
        for i in range(NSUB):
            if i > 0:
                cp_wq(i).start()
            cp_wg(i).start(); cp_wu(i).start(); cp_wd(i).start(); cp_wo(i).start()

        def init(k, carry):
            z_s[k] = 0
            st_v[k, pl.ds(0, 40), :] = jnp.zeros((40, TQ), _F32)
            st_v[k, pl.ds(40, 8), :] = jnp.full((8, TQ), -jnp.inf, _F32)
            return carry
        lax.fori_loop(0, len(units), init, 0)
        cp_wk().wait(); cp_wv().wait(); cp_gw().wait()
        gw8 = gw_v[...].astype(_F32)
        gwrow = jnp.concatenate([gw8[r:r + 1, :] for r in range(8)], axis=1)
        wkv_v[pl.ds(2 * DH, 16), :] = jnp.broadcast_to(gwrow, (16, D)).astype(_BF16)
        if PLOOP:
            cp_wq(0).wait()

            def pbody(blk, carry):
                cp_x(blk).wait()
                pr = [P(kv_chunk, blk)] + [P(q_proj, 0, pl.multiple_of(blk * TQ, TQ), blk, g) for g in range(NG)]
                for k in [(0, 1, 2), (1, 0, 2), (1, 2, 0)][PLOOP - 1]:
                    pr[k]()
                return carry
            lax.fori_loop(0, 2, pbody, 0)
        else:
            cp_x(0).wait()
            kv_chunk(0)
            cp_wq(0).wait()
            for g in range(NG):
                q_proj(0, 0, 0, g)
            cp_x(1).wait()
            kv_chunk(1)
            for g in range(NG):
                q_proj(0, TQ, 1, g)

        def group(att, keys, stk, lag, sched, order, last):
            def pre(key, c):
                if c == 0:
                    k = stk(key)
                    att.st[key] = (st_v[k, pl.ds(40, 1), :], st_v[k, pl.ds(32, 8), :], st_v[k, pl.ds(0, 32), :])

            def post(key, c):
                if c == CPG - 1 and not last:
                    k = stk(key)
                    m, l, o = att.st[key]
                    st_v[k, pl.ds(0, 32), :] = o
                    st_v[k, pl.ds(32, 8), :] = l
                    st_v[k, pl.ds(40, 8), :] = jnp.broadcast_to(m, (8, TQ))
            run(att, [(key, c) for key in keys for c in range(CPG)], lag, sched, order, pre=pre, post=post)

        if not SKIP1:
            def gbody(j, carry):
                c0 = 2 * j + 2
                cp_x(c0).wait()
                cp_x(c0 + 1).wait()
                ng = len(units) * CPG
                att = Attn(pl.multiple_of(j * KG, KG), CPG, qpre=units if QPRE0 else (), qz=QZG)
                sch = {}
                sch.setdefault(ng - 1 + KV0, []).append(P(kv_chunk, c0))
                sch.setdefault(ng - 1 + KV1, []).append(P(kv_chunk, c0 + 1))
                group(att, units, units.index, LAG0, sch, ["qpd", "pqd", "qdp"][ORD0], False)
                return carry
            lax.fori_loop(0, S // KG - 1, gbody, 0)

            def dbody(blk, carry):
                row0 = pl.multiple_of(blk * TQ, TQ)

                @pl.when(blk == 0)
                def _():
                    wait_view(wgu_v.at[0], s1 + 1)
                    wait_view(wdo_v.at[0], s1 + 2)
                att = Attn(S - KG, qslot=lambda _: blk, qpre=units[:HPS] if QPRE0 else (), qz=QZD)
                dn = Dense(0, row0, lambda k, u: att.final((0, u)), True)
                gu = dn.gu()
                g_fill(blk)
                sch = {}
                for k in range(DG):
                    sch.setdefault(k * DSP, []).append(gu[k])
                for k in range(1, NXC // 2):
                    sch.setdefault(k * DSP * 2, []).append(P(g_fill, blk + 2 * k))
                group(att, units[:HPS], lambda key: blk * HPS + key[1], LAG, sch, "qdp", True)
                qn = [P(q_proj, 0, row0 + 2 * TQ, blk, g) for g in range(NG)]
                for fn in gu[DG:DG + 1] + qn + gu[DG + 1:] + dn.downs():
                    fn()
                return carry
            lax.fori_loop(0, 2, dbody, 0)

        def body(t, carry):
            sub = lax.shift_right_logical(t, 2)
            pb = lax.bitwise_and(t, NPAIR - 1)

            @pl.when(t == NPAIR - 1)
            def _():
                for k, buf in enumerate((wq_v, wgu_v, wdo_v)):
                    wait_view(buf.at[pl.ds(1, NSUB - 1)], s1 + 3 + k)

            row0 = pl.multiple_of(pb * (2 * TQ), 2 * TQ)
            tn = jnp.minimum(t + 1, NSTEP - 1)
            nrow0 = pl.multiple_of(lax.bitwise_and(tn, NPAIR - 1) * (2 * TQ), 2 * TQ)
            if PROF:
                with jax.named_scope("other"):
                    uniform(sub, row0, lax.shift_right_logical(tn, 2), nrow0)
            else:
                uniform(sub, row0, lax.shift_right_logical(tn, 2), nrow0)
            return carry

        if not SKIPU:
            lax.fori_loop(1, NSTEP, body, 0)
        cp(out_v, out_hbm, sems.at[s_out]).wait()

    scratch = [
        pltpu.VMEM((S, D), _BF16),
        pltpu.VMEM((NSUB, D, QS), _BF16),
        pltpu.VMEM((2 * DH + 16, D), _BF16),
        pltpu.VMEM((8, 128), _BF16),
        pltpu.VMEM((NSUB, 2, D, FS), _BF16),
        pltpu.VMEM((NSUB, FS + QS, D), _BF16),
        pltpu.VMEM((S // 2, DH), jnp.uint32),
        pltpu.VMEM((NXC, DH // 2, XC), jnp.uint32),
        pltpu.VMEM((NXC, 8, XC), _F32),
        pltpu.VMEM((S, 128), _F32),
        pltpu.VMEM((2, NG, 64, TQ), jnp.uint32),
        pltpu.VMEM((S, D), _F32),
        pltpu.VMEM((S, D), _BF16),
        pltpu.VMEM((2 * HPS, 48, TQ), _F32),
        pltpu.SMEM((NKC,), jnp.int32),
        pltpu.SemaphoreType.DMA((NXC + 3 + 6 + 1,)),
    ]
    return kernel, scratch


def _build(**kw):
    any_spec = pl.BlockSpec(memory_space=pl.ANY)
    kernel, scratch = make_kernel(**kw)

    @jax.jit
    def fn(A_x, A_wq, A_wk, A_wv, A_wo, B_x, B_W_gate, B_W_up, B_W_down, gate_w):
        out = pl.pallas_call(
            kernel,
            in_specs=[any_spec] * 9,
            out_specs=any_spec,
            out_shape=jax.ShapeDtypeStruct((S, D), _BF16),
            scratch_shapes=scratch,
            compiler_params=pltpu.CompilerParams(vmem_limit_bytes=100 * 1024 * 1024),
            name="gmix",
        )(A_x.reshape(S, D), A_wq, A_wk.T, A_wv.T, A_wo, B_W_gate, B_W_up, B_W_down,
          gate_w.reshape(8, 128))
        return out.reshape(1, S, D)
    return fn


pallas_gated_mix__grouped_kv_mqa__glu_gated_reglu__prompt_kernel = _build()
```

```python
import functools
import math

import jax
import jax.numpy as jnp
from jax import lax
from jax.experimental import pallas as pl
from jax.experimental.pallas import tpu as pltpu

S = 2048
D = 1024
H = 32
DH = 32
F = 3584
TQ = 256
NB = S // TQ
XC = 256
NXC = S // XC
NSUB = 4
HPS = H // NSUB
FS = F // NSUB
QS = D // NSUB
NG = QS // 128
NF = FS // 128
KC = 128
NKC = S // KC
NPAIR = NB // 2
NSTEP = NSUB * NPAIR
KG = 512
CPG = KG // KC

LAG = 4
LAG0 = 6
QR = NKC

_NT = (((1,), (1,)), ((), ()))
_F32 = jnp.float32
_BF16 = jnp.bfloat16
_QSCALE = (DH ** -0.5) * math.log2(math.e)
_P = functools.partial


def _dot(a, b):
    return jnp.dot(a, b, preferred_element_type=_F32)


def _pack(a):
    return pltpu.bitcast(a, jnp.uint32)


def _unpack(a):
    return pltpu.bitcast(a, _BF16)


def _kernel(x_hbm, wq_hbm, wkt_hbm, wvt_hbm, wo_hbm, wg_hbm, wu_hbm, wd_hbm, gw_hbm,
            out_hbm,
            x_v, wq_v, wkv_v, gw_v, wgu_v, wdo_v,
            k_v, vt_v, lg_v, g_v, q_v, acc_v, out_v, st_v, z_s, sems):
    cp = pltpu.make_async_copy
    cp_x = lambda c: cp(x_hbm.at[pl.ds(c * XC, XC), :], x_v.at[pl.ds(c * XC, XC), :], sems.at[c])
    s0 = NXC
    cp_wk = lambda: cp(wkt_hbm, wkv_v.at[pl.ds(0, DH), :], sems.at[s0])
    cp_wv = lambda: cp(wvt_hbm, wkv_v.at[pl.ds(DH, DH), :], sems.at[s0 + 1])
    cp_gw = lambda: cp(gw_hbm, gw_v, sems.at[s0 + 2])
    s1 = s0 + 3
    sx = lambda i: 0 if i == 0 else 3
    cp_wq = lambda i: cp(wq_hbm.at[:, pl.ds(i * QS, QS)], wq_v.at[i], sems.at[s1 + sx(i)])
    cp_wg = lambda i: cp(wg_hbm.at[:, pl.ds(i * FS, FS)], wgu_v.at[i, 0], sems.at[s1 + 1 + sx(i)])
    cp_wu = lambda i: cp(wu_hbm.at[:, pl.ds(i * FS, FS)], wgu_v.at[i, 1], sems.at[s1 + 1 + sx(i)])
    cp_wd = lambda i: cp(wd_hbm.at[pl.ds(i * FS, FS), :], wdo_v.at[i, pl.ds(0, FS), :],
                         sems.at[s1 + 2 + sx(i)])
    cp_wo = lambda i: cp(wo_hbm.at[pl.ds(i * QS, QS), :], wdo_v.at[i, pl.ds(FS, QS), :],
                         sems.at[s1 + 2 + sx(i)])
    s_out = s1 + 6

    def wait_view(view, k):
        cp(view, view, sems.at[k]).wait()

    def kv_chunk(c):
        xc = x_v[pl.ds(pl.multiple_of(c * XC, XC), XC), :]
        rt = lax.dot_general(wkv_v[...], xc, _NT, preferred_element_type=_F32)
        k_v[pl.ds(pl.multiple_of(c * (XC // 2), XC // 2), XC // 2), :] = _pack(rt[0:DH, :].T.astype(_BF16))
        vt_v[c] = _pack(rt[DH:2 * DH, :].astype(_BF16))
        lg_v[c] = rt[2 * DH:2 * DH + 8, :]

    def g_fill(c):
        sg = jax.nn.sigmoid(lg_v[c])
        g_v[pl.ds(pl.multiple_of(c * XC, XC), XC), :] = jnp.concatenate([sg] * 16, axis=0).T

    pending_q = []

    def q_proj(slot, rows, blk, g, nb, rep):
        r = _dot(x_v[pl.ds(rows, nb * TQ), :], wq_v[slot, :, pl.ds(g * 128, 128)])
        for k in range(nb):
            qt = _pack((r[k * TQ:(k + 1) * TQ] * _QSCALE).T.astype(_BF16))
            for c in range(rep):
                q_v[c, blk + k, g] = qt
            if rep > 1:
                pending_q.extend(qt[16 * j:16 * (j + 1)] for j in range(4))

    def pace(tot):
        parts = []
        seg = tot.shape[0] // 4
        for k in range(4):
            part = tot[k * seg:(k + 1) * seg]
            if pending_q:
                qt = pltpu.bitcast(pending_q.pop(0), _F32)
                qt = jnp.concatenate([qt[:, :128], qt[:, 128:]], axis=0)
                part = jnp.concatenate([jnp.where(z_s[0] == 1, qt, part[:32]), part[32:]], axis=0)
            parts.append(part)
        return jnp.concatenate(parts, axis=0)

    class Attn:
        def __init__(self, kbase=0, preload=0, qslot=lambda blk: blk, qr=1):
            self.kbase, self.qslot, self.qr = kbase, qslot, qr
            self.s, self.st = {}, {}
            self.kc = {c: self.load_k(c) for c in range(preload)}
            self.vc = {c: self.load_v(c) for c in range(preload)}

        def load_k(self, c):
            h0 = self.kbase // 2 + c * (KC // 2)
            if not isinstance(h0, int):
                h0 = pl.multiple_of(h0, KC // 2)
            return _unpack(k_v[pl.ds(h0, KC // 2), :])

        def load_v(self, c):
            return _unpack(vt_v[self.kbase // XC + (c * KC) // XC, :, pl.ds((c * KC) % XC, KC)])

        def qk(self, key, c):
            blk, u = key
            kk = self.kc[c] if c in self.kc else self.load_k(c)
            qt = _unpack(q_v[c % self.qr, self.qslot(blk), u // 4, pl.ds((u % 4) * 16, 16), :])
            self.s[(key, c)] = _dot(kk, qt)

        def proc(self, key, c):
            s = self.s.pop((key, c))
            mc = jnp.max(jnp.max(s.reshape(KC // 8, 8, TQ), axis=0), axis=0, keepdims=True)
            prev = self.st.get(key)
            if prev is None:
                m = mc
            else:
                m0, l0, o0 = prev
                m = jnp.maximum(m0, mc)
                alpha = jnp.exp2(m0 - m)
            p = jnp.exp2(s - m)
            l = jnp.sum(p.reshape(KC // 8, 8, TQ), axis=0)
            vt = self.vc[c] if c in self.vc else self.load_v(c)
            o = _dot(vt, p.astype(_BF16))
            if prev is not None:
                l = l0 * alpha + l
                o = o0 * alpha + o
            self.st[key] = (m, l, o)

        def final(self, key):
            _, l, o = self.st[key]
            return o * (1.0 / jnp.sum(l, axis=0, keepdims=True))

    class Dense:
        def __init__(self, sub, row0, get_ot, first, nb):
            self.sub, self.row0, self.get_ot, self.first = sub, row0, get_ot, first
            self.nb, self.m = nb, nb * TQ
            self.part, self.hs, self.og, self.g = {}, {}, {}, None

        def gb(self):
            if self.g is None:
                self.g = g_v[pl.ds(self.row0, self.m), :]
            return self.g

        def gate(self, f):
            r = _dot(x_v[pl.ds(self.row0, self.m), :], wgu_v[self.sub, 0, :, pl.ds(f * 128, 128)])
            self.part[f] = jnp.maximum(r, 0.0) * (1.0 - self.gb())

        def up(self, f):
            r = _dot(x_v[pl.ds(self.row0, self.m), :], wgu_v[self.sub, 1, :, pl.ds(f * 128, 128)])
            self.hs[f] = (self.part.pop(f) * r).astype(_BF16)

        def gu(self):
            return [_P(fn, f) for f in range(NF) for fn in (self.gate, self.up)]

        def get_o(self, g):
            if g not in self.og:
                o4 = [jnp.concatenate([self.get_ot(k, 4 * g + j) for j in range(4)], axis=0).T
                      for k in range(self.nb)]
                self.og[g] = (jnp.concatenate(o4, axis=0) * self.gb()).astype(_BF16)
            return self.og[g]

        def down(self, n):
            cols = pl.ds(n * 128, 128)
            rows = pl.ds(self.row0, self.m)
            lhs = [self.hs[i] for i in range(NF)] + [self.get_o(i) for i in range(NG)]
            tot = _dot(jnp.concatenate(lhs, axis=1), wdo_v[self.sub, :, cols])
            if n >= 3 and pending_q:
                tot = pace(tot)
            if self.first:
                acc_v[rows, cols] = tot
            else:
                tot = jnp.where(self.sub == 0, 0.0, acc_v[rows, cols]) + tot
                acc_v[rows, cols] = tot
                out_v[rows, cols] = tot.astype(_BF16)

                @pl.when(self.sub == NSUB - 1)
                def _():
                    cp(out_v.at[rows, cols], out_hbm.at[rows, cols], sems.at[s_out]).start()

        def downs(self):
            return [_P(self.down, n) for n in range(D // 128)]

    def run(att, steps, lag, sched, order, pre=None, post=None):
        n = len(steps)
        for i in range(n + lag):
            if i >= lag and pre is not None:
                pre(*steps[i - lag])
            for what in order:
                if what == "q" and i < n:
                    att.qk(*steps[i])
                elif what == "p" and i >= lag:
                    att.proc(*steps[i - lag])
                elif what == "d":
                    for fn in sched.get(i, []):
                        fn()
            if i >= lag and post is not None:
                post(*steps[i - lag])

    units = [(blk, u) for blk in range(2) for u in range(HPS)]

    cp_x(0).start()
    cp_wk().start()
    cp_wv().start()
    cp_gw().start()
    cp_wq(0).start()
    for c in range(1, NXC):
        cp_x(c).start()
    for i in range(NSUB):
        if i > 0:
            cp_wq(i).start()
        cp_wg(i).start()
        cp_wu(i).start()
        cp_wd(i).start()
        cp_wo(i).start()

    def init(k, carry):
        z_s[k] = 0
        st_v[k, pl.ds(0, 40), :] = jnp.zeros((40, TQ), _F32)
        st_v[k, pl.ds(40, 8), :] = jnp.full((8, TQ), -jnp.inf, _F32)
        return carry
    lax.fori_loop(0, len(units), init, 0)
    cp_wk().wait()
    cp_wv().wait()
    cp_gw().wait()
    gw8 = gw_v[...].astype(_F32)
    gwrow = jnp.concatenate([gw8[r:r + 1, :] for r in range(8)], axis=1)
    wkv_v[pl.ds(2 * DH, 16), :] = jnp.broadcast_to(gwrow, (16, D)).astype(_BF16)
    cp_wq(0).wait()

    def pbody(blk, carry):
        cp_x(blk).wait()
        kv_chunk(blk)
        for g in range(NG):
            q_proj(0, pl.multiple_of(blk * TQ, TQ), blk, g, 1, 1)
        return carry
    lax.fori_loop(0, 2, pbody, 0)

    def group(att, keys, stk, lag, sched, last):
        def pre(key, c):
            if c == 0:
                k = stk(key)
                att.st[key] = (st_v[k, pl.ds(40, 1), :], st_v[k, pl.ds(32, 8), :], st_v[k, pl.ds(0, 32), :])

        def post(key, c):
            if c == CPG - 1 and not last:
                k = stk(key)
                m, l, o = att.st[key]
                st_v[k, pl.ds(0, 32), :] = o
                st_v[k, pl.ds(32, 8), :] = l
                st_v[k, pl.ds(40, 8), :] = jnp.broadcast_to(m, (8, TQ))
        run(att, [(key, c) for key in keys for c in range(CPG)], lag, sched, "qdp", pre, post)

    def gbody(j, carry):
        c0 = 2 * j + 2
        cp_x(c0).wait()
        cp_x(c0 + 1).wait()
        att = Attn(pl.multiple_of(j * KG, KG), CPG)
        sched = {2: [_P(kv_chunk, c0)], len(units) * CPG - 1: [_P(kv_chunk, c0 + 1)]}
        group(att, units, units.index, LAG0, sched, False)
        return carry
    lax.fori_loop(0, S // KG - 1, gbody, 0)

    def dbody(blk, carry):
        row0 = pl.multiple_of(blk * TQ, TQ)

        @pl.when(blk == 0)
        def _():
            wait_view(wgu_v.at[0], s1 + 1)
            wait_view(wdo_v.at[0], s1 + 2)
        att = Attn(S - KG, qslot=lambda _: blk)
        dn = Dense(0, row0, lambda k, u: att.final((0, u)), True, 1)
        gu = dn.gu()
        g_fill(blk)
        sched = {4 * k: [gu[k]] for k in range(9)}
        for k in range(1, NXC // 2):
            sched[8 * k].append(_P(g_fill, blk + 2 * k))
        group(att, units[:HPS], lambda key: blk * HPS + key[1], LAG, sched, True)
        qn = [_P(q_proj, 0, row0 + 2 * TQ, blk, g, 1, QR) for g in range(NG)]
        for fn in gu[9:10] + qn + gu[10:] + dn.downs():
            fn()
        return carry
    lax.fori_loop(0, 2, dbody, 0)

    def body(t, carry):
        sub = lax.shift_right_logical(t, 2)

        @pl.when(t == NPAIR - 1)
        def _():
            for k, buf in enumerate((wq_v, wgu_v, wdo_v)):
                wait_view(buf.at[pl.ds(1, NSUB - 1)], s1 + 3 + k)

        row0 = pl.multiple_of(lax.bitwise_and(t, NPAIR - 1) * (2 * TQ), 2 * TQ)
        tn = jnp.minimum(t + 1, NSTEP - 1)
        nsub = lax.shift_right_logical(tn, 2)
        nrow0 = pl.multiple_of(lax.bitwise_and(tn, NPAIR - 1) * (2 * TQ), 2 * TQ)

        att = Attn(qr=QR)
        steps = [(key, c) for key in units for c in range(NKC)]
        n = len(steps)
        dn = Dense(sub, row0, lambda k, u: att.final((k, u)), False, 2)
        gu = dn.gu()
        qn = [_P(q_proj, nsub, nrow0, 0, g, 2, QR) for g in range(NG)]
        sched = {2 * ((k * (n // 2)) // len(gu)): [fn] for k, fn in enumerate(gu)}
        sched[n - 1] = [qn[0]]
        run(att, steps, LAG, sched, "qpd")
        for fn in qn[1:] + dn.downs():
            fn()
        return carry
    lax.fori_loop(1, NSTEP, body, 0)
    cp(out_v, out_hbm, sems.at[s_out]).wait()


_SCRATCH = [
    pltpu.VMEM((S, D), _BF16),
    pltpu.VMEM((NSUB, D, QS), _BF16),
    pltpu.VMEM((2 * DH + 16, D), _BF16),
    pltpu.VMEM((8, 128), _BF16),
    pltpu.VMEM((NSUB, 2, D, FS), _BF16),
    pltpu.VMEM((NSUB, FS + QS, D), _BF16),
    pltpu.VMEM((S // 2, DH), jnp.uint32),
    pltpu.VMEM((NXC, DH // 2, XC), jnp.uint32),
    pltpu.VMEM((NXC, 8, XC), _F32),
    pltpu.VMEM((S, 128), _F32),
    pltpu.VMEM((QR, 2, NG, 64, TQ), jnp.uint32),
    pltpu.VMEM((S, D), _F32),
    pltpu.VMEM((S, D), _BF16),
    pltpu.VMEM((2 * HPS, 48, TQ), _F32),
    pltpu.SMEM((2 * HPS,), jnp.int32),
    pltpu.SemaphoreType.DMA((NXC + 3 + 6 + 1,)),
]


@jax.jit
def pallas_gated_mix__grouped_kv_mqa__glu_gated_reglu__prompt_kernel(
    A_x: jax.Array,
    A_wq: jax.Array,
    A_wk: jax.Array,
    A_wv: jax.Array,
    A_wo: jax.Array,
    B_x: jax.Array,
    B_W_gate: jax.Array,
    B_W_up: jax.Array,
    B_W_down: jax.Array,
    gate_w: jax.Array,
):
    del B_x
    any_spec = pl.BlockSpec(memory_space=pl.ANY)
    out = pl.pallas_call(
        _kernel,
        in_specs=[any_spec] * 9,
        out_specs=any_spec,
        out_shape=jax.ShapeDtypeStruct((S, D), _BF16),
        scratch_shapes=_SCRATCH,
        compiler_params=pltpu.CompilerParams(vmem_limit_bytes=100 * 1024 * 1024),
        name="gmix",
    )(A_x.reshape(S, D), A_wq, A_wk.T, A_wv.T, A_wo, B_W_gate, B_W_up, B_W_down,
      gate_w.reshape(8, 128))
    return out.reshape(1, S, D)
```

```python
import functools
import math

import jax
import jax.numpy as jnp
from jax import lax
from jax.experimental import pallas as pl
from jax.experimental.pallas import tpu as pltpu

S = 2048
D = 1024
H = 32
DH = 32
F = 3584
TQ = 256
NB = S // TQ
XC = 256
NXC = S // XC
NSUB = 4
HPS = H // NSUB
FS = F // NSUB
QS = D // NSUB
NG = QS // 128
NF = FS // 128
KC = 128
NKC = S // KC
NPAIR = NB // 2
NSTEP = NSUB * NPAIR
KG = 512
CPG = KG // KC

LAG = 4
LAG0 = 6
QR = NKC

GU_POS = (0, 22, 32, 56, 74, 94, 104, 126, 148, 166, 182, 198, 214, 240)

_NT = (((1,), (1,)), ((), ()))
_F32 = jnp.float32
_BF16 = jnp.bfloat16
_QSCALE = (DH ** -0.5) * math.log2(math.e)
_P = functools.partial


def _dot(a, b):
    return jnp.dot(a, b, preferred_element_type=_F32)


def _pack(a):
    return pltpu.bitcast(a, jnp.uint32)


def _unpack(a):
    return pltpu.bitcast(a, _BF16)


def _kernel(x_hbm, wq_hbm, wkt_hbm, wvt_hbm, wo_hbm, wg_hbm, wu_hbm, wd_hbm, gw_hbm,
            out_hbm,
            x_v, wq_v, wgu_v, wdo_v,
            k_v, vt_v, lg_v, g_v, q_v, acc_v, out_v, st_v, wkv_v, gw_v, z_s, sems):
    cp = pltpu.make_async_copy
    cp_x = lambda c: cp(x_hbm.at[pl.ds(c * XC, XC), :], x_v.at[pl.ds(c * XC, XC), :], sems.at[c])
    s0 = NXC
    cp_wk = lambda: cp(wkt_hbm, wkv_v.at[pl.ds(0, DH), :], sems.at[s0])
    cp_wv = lambda: cp(wvt_hbm, wkv_v.at[pl.ds(DH, DH), :], sems.at[s0 + 1])
    cp_gw = lambda: cp(gw_hbm, gw_v, sems.at[s0 + 2])
    s1 = s0 + 3
    sx = lambda i: 0 if i == 0 else 3
    cp_wq = lambda i: cp(wq_hbm.at[:, pl.ds(i * QS, QS)], wq_v.at[i], sems.at[s1 + sx(i)])
    cp_wg = lambda i: cp(wg_hbm.at[:, pl.ds(i * FS, FS)], wgu_v.at[i, 0], sems.at[s1 + 1 + sx(i)])
    cp_wu = lambda i: cp(wu_hbm.at[:, pl.ds(i * FS, FS)], wgu_v.at[i, 1], sems.at[s1 + 1 + sx(i)])
    cp_wd = lambda i: cp(wd_hbm.at[pl.ds(i * FS, FS), :], wdo_v.at[i, pl.ds(0, FS), :],
                         sems.at[s1 + 2 + sx(i)])
    cp_wo = lambda i: cp(wo_hbm.at[pl.ds(i * QS, QS), :], wdo_v.at[i, pl.ds(FS, QS), :],
                         sems.at[s1 + 2 + sx(i)])
    s_out = s1 + 6

    def wait_view(view, k):
        cp(view, view, sems.at[k]).wait()

    def kv_chunk(c):
        xc = x_v[pl.ds(pl.multiple_of(c * XC, XC), XC), :]
        rt = lax.dot_general(wkv_v[...], xc, _NT, preferred_element_type=_F32)
        k_v[pl.ds(pl.multiple_of(c * (XC // 2), XC // 2), XC // 2), :] = _pack(rt[0:DH, :].T.astype(_BF16))
        vt_v[c] = _pack(rt[DH:2 * DH, :].astype(_BF16))
        lg_v[c, pl.ds(0, 8), :] = rt[2 * DH:2 * DH + 8, :]

    def g_fill(c):
        sg = jax.nn.sigmoid(lg_v[c, pl.ds(0, 8), :])
        g_v[pl.ds(pl.multiple_of(c * XC, XC), XC), :] = jnp.concatenate([sg] * 16, axis=0).T

    pending_q = []

    def q_proj(slot, rows, blk, g, nb, rep):
        r = _dot(x_v[pl.ds(rows, nb * TQ), :], wq_v[slot, :, pl.ds(g * 128, 128)])
        for k in range(nb):
            qt = _pack((r[k * TQ:(k + 1) * TQ] * _QSCALE).T.astype(_BF16))
            for c in range(rep):
                q_v[c, blk + k, g] = qt
            if rep > 1:
                pending_q.extend(qt[16 * j:16 * (j + 1)] for j in range(4))

    def pace(tot):
        parts = []
        seg = tot.shape[0] // 4
        for k in range(4):
            part = tot[k * seg:(k + 1) * seg]
            if pending_q:
                qt = pltpu.bitcast(pending_q.pop(0), _F32)
                qt = jnp.concatenate([qt[:, :128], qt[:, 128:]], axis=0)
                part = jnp.concatenate([jnp.where(z_s[0] == 1, qt, part[:32]), part[32:]], axis=0)
            parts.append(part)
        return jnp.concatenate(parts, axis=0)

    class Attn:
        def __init__(self, kbase=0, preload=0, qslot=lambda blk: blk, qr=1):
            self.kbase, self.qslot, self.qr = kbase, qslot, qr
            self.s, self.st = {}, {}
            self.kc = {c: self.load_k(c) for c in range(preload)}
            self.vc = {c: self.load_v(c) for c in range(preload)}

        def load_k(self, c):
            h0 = self.kbase // 2 + c * (KC // 2)
            if not isinstance(h0, int):
                h0 = pl.multiple_of(h0, KC // 2)
            return _unpack(k_v[pl.ds(h0, KC // 2), :])

        def load_v(self, c):
            return _unpack(vt_v[self.kbase // XC + (c * KC) // XC, :, pl.ds((c * KC) % XC, KC)])

        def qk(self, key, c):
            blk, u = key
            kk = self.kc[c] if c in self.kc else self.load_k(c)
            qt = _unpack(q_v[c % self.qr, self.qslot(blk), u // 4, pl.ds((u % 4) * 16, 16), :])
            self.s[(key, c)] = _dot(kk, qt)

        def proc(self, key, c):
            s = self.s.pop((key, c))
            mc = jnp.max(jnp.max(s.reshape(KC // 8, 8, TQ), axis=0), axis=0, keepdims=True)
            prev = self.st.get(key)
            if prev is None:
                m = mc
            else:
                m0, l0, o0 = prev
                m = jnp.maximum(m0, mc)
                alpha = jnp.exp2(m0 - m)
            p = jnp.exp2(s - m)
            l = jnp.sum(p.reshape(KC // 8, 8, TQ), axis=0)
            vt = self.vc[c] if c in self.vc else self.load_v(c)
            o = _dot(vt, p.astype(_BF16))
            if prev is not None:
                l = l0 * alpha + l
                o = o0 * alpha + o
            self.st[key] = (m, l, o)

        def final(self, key):
            _, l, o = self.st[key]
            return o * (1.0 / jnp.sum(l, axis=0, keepdims=True))

    class Dense:
        def __init__(self, sub, row0, get_ot, first, nb):
            self.sub, self.row0, self.get_ot, self.first = sub, row0, get_ot, first
            self.nb, self.m = nb, nb * TQ
            self.part, self.hs, self.og, self.g = {}, {}, {}, None

        def gb(self):
            if self.g is None:
                self.g = g_v[pl.ds(self.row0, self.m), :]
            return self.g

        def gate(self, f):
            r = _dot(x_v[pl.ds(self.row0, self.m), :], wgu_v[self.sub, 0, :, pl.ds(f * 128, 128)])
            self.part[f] = jnp.maximum(r, 0.0) * (1.0 - self.gb())

        def up(self, f):
            r = _dot(x_v[pl.ds(self.row0, self.m), :], wgu_v[self.sub, 1, :, pl.ds(f * 128, 128)])
            self.hs[f] = (self.part.pop(f) * r).astype(_BF16)

        def gu(self):
            return [_P(fn, f) for f in range(NF) for fn in (self.gate, self.up)]

        def get_o(self, g):
            if g not in self.og:
                o4 = [jnp.concatenate([self.get_ot(k, 4 * g + j) for j in range(4)], axis=0).T
                      for k in range(self.nb)]
                self.og[g] = (jnp.concatenate(o4, axis=0) * self.gb()).astype(_BF16)
            return self.og[g]

        def down(self, n):
            cols = pl.ds(n * 128, 128)
            rows = pl.ds(self.row0, self.m)
            lhs = [self.hs[i] for i in range(NF)] + [self.get_o(i) for i in range(NG)]
            tot = _dot(jnp.concatenate(lhs, axis=1), wdo_v[self.sub, :, cols])
            if n >= 3 and pending_q:
                tot = pace(tot)
            if self.first:
                acc_v[rows, cols] = tot
            else:
                tot = jnp.where(self.sub == 0, 0.0, acc_v[rows, cols]) + tot
                acc_v[rows, cols] = tot
                out_v[rows, cols] = tot.astype(_BF16)

                @pl.when(self.sub == NSUB - 1)
                def _():
                    cp(out_v.at[rows, cols], out_hbm.at[rows, cols], sems.at[s_out]).start()

        def downs(self):
            return [_P(self.down, n) for n in range(D // 128)]

    def run(att, steps, lag, sched, order, pre=None, post=None):
        n = len(steps)
        for i in range(n + lag):
            if i >= lag and pre is not None:
                pre(*steps[i - lag])
            for what in order:
                if what == "q" and i < n:
                    att.qk(*steps[i])
                elif what == "p" and i >= lag:
                    att.proc(*steps[i - lag])
                elif what == "d":
                    for fn in sched.get(i, []):
                        fn()
            if i >= lag and post is not None:
                post(*steps[i - lag])

    units = [(blk, u) for blk in range(2) for u in range(HPS)]

    cp_x(0).start()
    cp_wk().start()
    cp_wv().start()
    cp_gw().start()
    cp_wq(0).start()
    for c in range(1, NXC):
        cp_x(c).start()
    for i in range(NSUB):
        if i > 0:
            cp_wq(i).start()
        cp_wg(i).start()
        cp_wu(i).start()
        cp_wd(i).start()
        cp_wo(i).start()

    def init(k, carry):
        z_s[k] = 0
        st_v[k, pl.ds(0, 40), :] = jnp.zeros((40, TQ), _F32)
        st_v[k, pl.ds(40, 8), :] = jnp.full((8, TQ), -jnp.inf, _F32)
        return carry
    lax.fori_loop(0, len(units), init, 0)
    cp_wk().wait()
    cp_wv().wait()
    cp_gw().wait()
    gw8 = gw_v[...].astype(_F32)
    gwrow = jnp.concatenate([gw8[r:r + 1, :] for r in range(8)], axis=1)
    wkv_v[pl.ds(2 * DH, 16), :] = jnp.broadcast_to(gwrow, (16, D)).astype(_BF16)
    cp_wq(0).wait()

    def pbody(blk, carry):
        cp_x(blk).wait()
        kv_chunk(blk)
        for g in range(NG):
            q_proj(0, pl.multiple_of(blk * TQ, TQ), blk, g, 1, 1)
        return carry
    lax.fori_loop(0, 2, pbody, 0)

    def group(att, keys, stk, lag, sched, last):
        def pre(key, c):
            if c == 0:
                k = stk(key)
                att.st[key] = (st_v[k, pl.ds(40, 1), :], st_v[k, pl.ds(32, 8), :], st_v[k, pl.ds(0, 32), :])

        def post(key, c):
            if c == CPG - 1 and not last:
                k = stk(key)
                m, l, o = att.st[key]
                st_v[k, pl.ds(0, 32), :] = o
                st_v[k, pl.ds(32, 8), :] = l
                st_v[k, pl.ds(40, 8), :] = jnp.broadcast_to(m, (8, TQ))
        run(att, [(key, c) for key in keys for c in range(CPG)], lag, sched, "qdp", pre, post)

    def gbody(j, carry):
        c0 = 2 * j + 2
        cp_x(c0).wait()
        cp_x(c0 + 1).wait()
        att = Attn(pl.multiple_of(j * KG, KG), CPG)
        sched = {2: [_P(kv_chunk, c0)], len(units) * CPG - 1: [_P(kv_chunk, c0 + 1)]}
        group(att, units, units.index, LAG0, sched, False)
        return carry
    lax.fori_loop(0, S // KG - 1, gbody, 0)

    def dbody(blk, carry):
        row0 = pl.multiple_of(blk * TQ, TQ)

        @pl.when(blk == 0)
        def _():
            wait_view(wgu_v.at[0], s1 + 1)
            wait_view(wdo_v.at[0], s1 + 2)
        att = Attn(S - KG, qslot=lambda _: blk)
        dn = Dense(0, row0, lambda k, u: att.final((0, u)), True, 1)
        gu = dn.gu()
        g_fill(blk)
        sched = {4 * k: [gu[k]] for k in range(9)}
        for k in range(1, NXC // 2):
            sched[8 * k].append(_P(g_fill, blk + 2 * k))
        group(att, units[:HPS], lambda key: blk * HPS + key[1], LAG, sched, True)
        qn = [_P(q_proj, 0, row0 + 2 * TQ, blk, g, 1, QR) for g in range(NG)]
        for fn in gu[9:10] + qn + gu[10:] + dn.downs():
            fn()
        return carry
    lax.fori_loop(0, 2, dbody, 0)

    def body(t, carry):
        sub = lax.shift_right_logical(t, 2)

        @pl.when(t == NPAIR - 1)
        def _():
            for k, buf in enumerate((wq_v, wgu_v, wdo_v)):
                wait_view(buf.at[pl.ds(1, NSUB - 1)], s1 + 3 + k)

        row0 = pl.multiple_of(lax.bitwise_and(t, NPAIR - 1) * (2 * TQ), 2 * TQ)
        tn = jnp.minimum(t + 1, NSTEP - 1)
        nsub = lax.shift_right_logical(tn, 2)
        nrow0 = pl.multiple_of(lax.bitwise_and(tn, NPAIR - 1) * (2 * TQ), 2 * TQ)

        att = Attn(qr=QR)
        steps = [(key, c) for key in units for c in range(NKC)]
        n = len(steps)
        dn = Dense(sub, row0, lambda k, u: att.final((k, u)), False, 2)
        gu = dn.gu()
        qn = [_P(q_proj, nsub, nrow0, 0, g, 2, QR) for g in range(NG)]
        sched = {pos: [fn] for pos, fn in zip(GU_POS, gu, strict=True)}
        sched[n - 1] = [qn[0]]
        run(att, steps, LAG, sched, "qpd")
        for fn in qn[1:] + dn.downs():
            fn()
        return carry
    lax.fori_loop(1, NSTEP, body, 0)
    cp(out_v, out_hbm, sems.at[s_out]).wait()


_SCRATCH = [
    pltpu.VMEM((S, D), _BF16),
    pltpu.VMEM((NSUB, D, QS), _BF16),
    pltpu.VMEM((NSUB, 2, D, FS), _BF16),
    pltpu.VMEM((NSUB, FS + QS, D), _BF16),
    pltpu.VMEM((S // 2, DH), jnp.uint32),
    pltpu.VMEM((NXC, DH // 2, XC), jnp.uint32),
    pltpu.VMEM((NXC, 16, XC), _F32),
    pltpu.VMEM((S, 128), _F32),
    pltpu.VMEM((QR, 2, NG, 64, TQ), jnp.uint32),
    pltpu.VMEM((S, D), _F32),
    pltpu.VMEM((S, D), _BF16),
    pltpu.VMEM((2 * HPS, 48, TQ), _F32),
    pltpu.VMEM((2 * DH + 16, D), _BF16),
    pltpu.VMEM((8, 128), _BF16),
    pltpu.SMEM((2 * HPS,), jnp.int32),
    pltpu.SemaphoreType.DMA((NXC + 3 + 6 + 1,)),
]


@jax.jit
def pallas_gated_mix__grouped_kv_mqa__glu_gated_reglu__prompt_kernel(
    A_x: jax.Array,
    A_wq: jax.Array,
    A_wk: jax.Array,
    A_wv: jax.Array,
    A_wo: jax.Array,
    B_x: jax.Array,
    B_W_gate: jax.Array,
    B_W_up: jax.Array,
    B_W_down: jax.Array,
    gate_w: jax.Array,
):
    del B_x
    any_spec = pl.BlockSpec(memory_space=pl.ANY)
    out = pl.pallas_call(
        _kernel,
        in_specs=[any_spec] * 9,
        out_specs=any_spec,
        out_shape=jax.ShapeDtypeStruct((S, D), _BF16),
        scratch_shapes=_SCRATCH,
        compiler_params=pltpu.CompilerParams(vmem_limit_bytes=100 * 1024 * 1024),
        name="gmix",
    )(A_x.reshape(S, D), A_wq, A_wk.T, A_wv.T, A_wo, B_W_gate, B_W_up, B_W_down,
      gate_w.reshape(8, 128))
    return out.reshape(1, S, D)
```

```python
import functools
import math

import jax
import jax.numpy as jnp
from jax import lax
from jax.experimental import pallas as pl
from jax.experimental.pallas import tpu as pltpu

S = 2048
D = 1024
H = 32
DH = 32
F = 3584
TQ = 256
NB = S // TQ
XC = 256
NXC = S // XC
NSUB = 4
HPS = H // NSUB
FS = F // NSUB
QS = D // NSUB
NG = QS // 128
NF = FS // 128
KC = 128
NKC = S // KC
NPAIR = NB // 2
NSTEP = NSUB * NPAIR
KG = 512
CPG = KG // KC

LAG = 4
LAG0 = 6
QR = NKC

GU_POS = (0, 22, 32, 56, 74, 94, 104, 126, 148, 166, 182, 200, 214, 240)

_NT = (((1,), (1,)), ((), ()))
_F32 = jnp.float32
_BF16 = jnp.bfloat16
_QSCALE = (DH ** -0.5) * math.log2(math.e)
_P = functools.partial


def _dot(a, b):
    return jnp.dot(a, b, preferred_element_type=_F32)


def _pack(a):
    return pltpu.bitcast(a, jnp.uint32)


def _unpack(a):
    return pltpu.bitcast(a, _BF16)


def _kernel(x_hbm, wq_hbm, wkt_hbm, wvt_hbm, wo_hbm, wg_hbm, wu_hbm, wd_hbm, gw_hbm,
            out_hbm,
            x_v, wq_v, wgu_v, wdo_v,
            k_v, vt_v, lg_v, g_v, q_v, acc_v, out_v, st_v, wkv_v, gw_v, z_s, sems):
    cp = pltpu.make_async_copy
    cp_x = lambda c: cp(x_hbm.at[pl.ds(c * XC, XC), :], x_v.at[pl.ds(c * XC, XC), :], sems.at[c])
    s0 = NXC
    cp_wk = lambda: cp(wkt_hbm, wkv_v.at[pl.ds(0, DH), :], sems.at[s0])
    cp_wv = lambda: cp(wvt_hbm, wkv_v.at[pl.ds(DH, DH), :], sems.at[s0 + 1])
    cp_gw = lambda: cp(gw_hbm, gw_v, sems.at[s0 + 2])
    s1 = s0 + 3
    sx = lambda i: 0 if i == 0 else 3
    cp_wq = lambda i: cp(wq_hbm.at[:, pl.ds(i * QS, QS)], wq_v.at[i], sems.at[s1 + sx(i)])
    cp_wg = lambda i: cp(wg_hbm.at[:, pl.ds(i * FS, FS)], wgu_v.at[i, 0], sems.at[s1 + 1 + sx(i)])
    cp_wu = lambda i: cp(wu_hbm.at[:, pl.ds(i * FS, FS)], wgu_v.at[i, 1], sems.at[s1 + 1 + sx(i)])
    cp_wd = lambda i: cp(wd_hbm.at[pl.ds(i * FS, FS), :], wdo_v.at[i, pl.ds(0, FS), :],
                         sems.at[s1 + 2 + sx(i)])
    cp_wo = lambda i: cp(wo_hbm.at[pl.ds(i * QS, QS), :], wdo_v.at[i, pl.ds(FS, QS), :],
                         sems.at[s1 + 2 + sx(i)])
    s_out = s1 + 6

    def wait_view(view, k):
        cp(view, view, sems.at[k]).wait()

    def kv_chunk(c):
        xc = x_v[pl.ds(pl.multiple_of(c * XC, XC), XC), :]
        rt = lax.dot_general(wkv_v[...], xc, _NT, preferred_element_type=_F32)
        k_v[pl.ds(pl.multiple_of(c * (XC // 2), XC // 2), XC // 2), :] = _pack(rt[0:DH, :].T.astype(_BF16))
        vt_v[c] = _pack(rt[DH:2 * DH, :].astype(_BF16))
        lg_v[c, pl.ds(0, 8), :] = rt[2 * DH:2 * DH + 8, :]

    def g_fill(c):
        sg = jax.nn.sigmoid(lg_v[c, pl.ds(0, 8), :])
        g_v[pl.ds(pl.multiple_of(c * XC, XC), XC), :] = jnp.concatenate([sg] * 16, axis=0).T

    pending_q = []

    def q_proj(slot, rows, blk, g, nb, rep):
        r = _dot(x_v[pl.ds(rows, nb * TQ), :], wq_v[slot, :, pl.ds(g * 128, 128)])
        for k in range(nb):
            qt = _pack((r[k * TQ:(k + 1) * TQ] * _QSCALE).T.astype(_BF16))
            for c in range(rep):
                q_v[c, blk + k, g] = qt
            if rep > 1:
                pending_q.extend(qt[16 * j:16 * (j + 1)] for j in range(4))

    def pace(tot):
        parts = []
        seg = tot.shape[0] // 4
        for k in range(4):
            part = tot[k * seg:(k + 1) * seg]
            if pending_q:
                qt = pltpu.bitcast(pending_q.pop(0), _F32)
                qt = jnp.concatenate([qt[:, :128], qt[:, 128:]], axis=0)
                part = jnp.concatenate([jnp.where(z_s[0] == 1, qt, part[:32]), part[32:]], axis=0)
            parts.append(part)
        return jnp.concatenate(parts, axis=0)

    class Attn:
        def __init__(self, kbase=0, preload=0, qslot=lambda blk: blk, qr=1):
            self.kbase, self.qslot, self.qr = kbase, qslot, qr
            self.s, self.st = {}, {}
            self.kc = {c: self.load_k(c) for c in range(preload)}
            self.vc = {c: self.load_v(c) for c in range(preload)}

        def load_k(self, c):
            h0 = self.kbase // 2 + c * (KC // 2)
            if not isinstance(h0, int):
                h0 = pl.multiple_of(h0, KC // 2)
            return _unpack(k_v[pl.ds(h0, KC // 2), :])

        def load_v(self, c):
            return _unpack(vt_v[self.kbase // XC + (c * KC) // XC, :, pl.ds((c * KC) % XC, KC)])

        def qk(self, key, c):
            blk, u = key
            kk = self.kc[c] if c in self.kc else self.load_k(c)
            qt = _unpack(q_v[c % self.qr, self.qslot(blk), u // 4, pl.ds((u % 4) * 16, 16), :])
            self.s[(key, c)] = _dot(kk, qt)

        def proc(self, key, c):
            s = self.s.pop((key, c))
            mc = jnp.max(jnp.max(s.reshape(KC // 8, 8, TQ), axis=0), axis=0, keepdims=True)
            prev = self.st.get(key)
            if prev is None:
                m = mc
            else:
                m0, l0, o0 = prev
                m = jnp.maximum(m0, mc)
                alpha = jnp.exp2(m0 - m)
            p = jnp.exp2(s - m)
            l = jnp.sum(p.reshape(KC // 8, 8, TQ), axis=0)
            vt = self.vc[c] if c in self.vc else self.load_v(c)
            o = _dot(vt, p.astype(_BF16))
            if prev is not None:
                l = l0 * alpha + l
                o = o0 * alpha + o
            self.st[key] = (m, l, o)

        def final(self, key):
            _, l, o = self.st[key]
            return o * (1.0 / jnp.sum(l, axis=0, keepdims=True))

    class Dense:
        def __init__(self, sub, row0, get_ot, first, nb):
            self.sub, self.row0, self.get_ot, self.first = sub, row0, get_ot, first
            self.nb, self.m = nb, nb * TQ
            self.part, self.hs, self.og, self.g = {}, {}, {}, None

        def gb(self):
            if self.g is None:
                self.g = g_v[pl.ds(self.row0, self.m), :]
            return self.g

        def gate(self, f):
            r = _dot(x_v[pl.ds(self.row0, self.m), :], wgu_v[self.sub, 0, :, pl.ds(f * 128, 128)])
            self.part[f] = jnp.maximum(r, 0.0) * (1.0 - self.gb())

        def up(self, f):
            r = _dot(x_v[pl.ds(self.row0, self.m), :], wgu_v[self.sub, 1, :, pl.ds(f * 128, 128)])
            self.hs[f] = (self.part.pop(f) * r).astype(_BF16)

        def gu(self):
            return [_P(fn, f) for f in range(NF) for fn in (self.gate, self.up)]

        def get_o(self, g):
            if g not in self.og:
                o4 = [jnp.concatenate([self.get_ot(k, 4 * g + j) for j in range(4)], axis=0).T
                      for k in range(self.nb)]
                self.og[g] = (jnp.concatenate(o4, axis=0) * self.gb()).astype(_BF16)
            return self.og[g]

        def down(self, n):
            cols = pl.ds(n * 128, 128)
            rows = pl.ds(self.row0, self.m)
            lhs = [self.hs[i] for i in range(NF)] + [self.get_o(i) for i in range(NG)]
            tot = _dot(jnp.concatenate(lhs, axis=1), wdo_v[self.sub, :, cols])
            if n >= (5 if self.first else 3) and pending_q:
                tot = pace(tot)
            if self.first:
                acc_v[rows, cols] = tot
            else:
                tot = jnp.where(self.sub == 0, 0.0, acc_v[rows, cols]) + tot
                acc_v[rows, cols] = tot
                out_v[rows, cols] = tot.astype(_BF16)

                @pl.when(self.sub == NSUB - 1)
                def _():
                    cp(out_v.at[rows, cols], out_hbm.at[rows, cols], sems.at[s_out]).start()

        def downs(self):
            return [_P(self.down, n) for n in range(D // 128)]

    def run(att, steps, lag, sched, order, pre=None, post=None):
        n = len(steps)
        for i in range(n + lag):
            if i >= lag and pre is not None:
                pre(*steps[i - lag])
            for what in order:
                if what == "q" and i < n:
                    att.qk(*steps[i])
                elif what == "p" and i >= lag:
                    att.proc(*steps[i - lag])
                elif what == "d":
                    for fn in sched.get(i, []):
                        fn()
            if i >= lag and post is not None:
                post(*steps[i - lag])

    units = [(blk, u) for blk in range(2) for u in range(HPS)]

    cp_x(0).start()
    cp_wk().start()
    cp_wv().start()
    cp_gw().start()
    cp_wq(0).start()
    for c in range(1, NXC):
        cp_x(c).start()
    for i in range(NSUB):
        if i > 0:
            cp_wq(i).start()
        cp_wg(i).start()
        cp_wu(i).start()
        cp_wd(i).start()
        cp_wo(i).start()

    def init(k, carry):
        z_s[k] = 0
        st_v[k, pl.ds(0, 40), :] = jnp.zeros((40, TQ), _F32)
        st_v[k, pl.ds(40, 8), :] = jnp.full((8, TQ), -jnp.inf, _F32)
        return carry
    lax.fori_loop(0, len(units), init, 0)
    cp_wk().wait()
    cp_wv().wait()
    cp_gw().wait()
    gw8 = gw_v[...].astype(_F32)
    gwrow = jnp.concatenate([gw8[r:r + 1, :] for r in range(8)], axis=1)
    wkv_v[pl.ds(2 * DH, 16), :] = jnp.broadcast_to(gwrow, (16, D)).astype(_BF16)
    cp_wq(0).wait()

    def pbody(blk, carry):
        cp_x(blk).wait()
        rows = pl.multiple_of(blk * TQ, TQ)
        q_proj(0, rows, blk, 0, 1, 1)
        kv_chunk(blk)
        q_proj(0, rows, blk, 1, 1, 1)
        return carry
    lax.fori_loop(0, 2, pbody, 0)

    def group(att, keys, stk, lag, sched, last):
        def pre(key, c):
            if c == 0:
                k = stk(key)
                att.st[key] = (st_v[k, pl.ds(40, 1), :], st_v[k, pl.ds(32, 8), :], st_v[k, pl.ds(0, 32), :])

        def post(key, c):
            if c == CPG - 1 and not last:
                k = stk(key)
                m, l, o = att.st[key]
                st_v[k, pl.ds(0, 32), :] = o
                st_v[k, pl.ds(32, 8), :] = l
                st_v[k, pl.ds(40, 8), :] = jnp.broadcast_to(m, (8, TQ))
        run(att, [(key, c) for key in keys for c in range(CPG)], lag, sched, "qdp", pre, post)

    def gbody(j, carry):
        c0 = 2 * j + 2
        cp_x(c0).wait()
        cp_x(c0 + 1).wait()
        att = Attn(pl.multiple_of(j * KG, KG), CPG)
        sched = {2: [_P(kv_chunk, c0)], len(units) * CPG - 1: [_P(kv_chunk, c0 + 1)]}
        group(att, units, units.index, LAG0, sched, False)
        return carry
    lax.fori_loop(0, S // KG - 1, gbody, 0)

    def dbody(blk, carry):
        row0 = pl.multiple_of(blk * TQ, TQ)

        @pl.when(blk == 0)
        def _():
            wait_view(wgu_v.at[0], s1 + 1)
            wait_view(wdo_v.at[0], s1 + 2)
        att = Attn(S - KG, qslot=lambda _: blk)
        dn = Dense(0, row0, lambda k, u: att.final((0, u)), True, 1)
        gu = dn.gu()
        g_fill(blk)
        sched = {3 * k: [gu[k]] for k in range(13)}
        for k in range(1, NXC // 2):
            sched.setdefault(8 * k, []).append(_P(g_fill, blk + 2 * k))
        group(att, units[:HPS], lambda key: blk * HPS + key[1], LAG0, sched, True)
        qn = [_P(q_proj, 0, row0 + 2 * TQ, blk, g, 1, QR) for g in range(NG)]
        for fn in gu[13:] + qn + dn.downs():
            fn()
        return carry
    lax.fori_loop(0, 2, dbody, 0)

    def body(t, carry):
        sub = lax.shift_right_logical(t, 2)

        @pl.when(t == NPAIR - 1)
        def _():
            for k, buf in enumerate((wq_v, wgu_v, wdo_v)):
                wait_view(buf.at[pl.ds(1, NSUB - 1)], s1 + 3 + k)

        row0 = pl.multiple_of(lax.bitwise_and(t, NPAIR - 1) * (2 * TQ), 2 * TQ)
        tn = jnp.minimum(t + 1, NSTEP - 1)
        nsub = lax.shift_right_logical(tn, 2)
        nrow0 = pl.multiple_of(lax.bitwise_and(tn, NPAIR - 1) * (2 * TQ), 2 * TQ)

        att = Attn(qr=QR)
        steps = [(key, c) for key in units for c in range(NKC)]
        n = len(steps)
        dn = Dense(sub, row0, lambda k, u: att.final((k, u)), False, 2)
        gu = dn.gu()
        qn = [_P(q_proj, nsub, nrow0, 0, g, 2, QR) for g in range(NG)]
        sched = {pos: [fn] for pos, fn in zip(GU_POS, gu, strict=True)}
        sched[n - 1] = [qn[0]]
        run(att, steps, LAG, sched, "qpd")
        for fn in qn[1:] + dn.downs():
            fn()
        return carry
    lax.fori_loop(1, NSTEP, body, 0)
    cp(out_v, out_hbm, sems.at[s_out]).wait()


_SCRATCH = [
    pltpu.VMEM((S, D), _BF16),
    pltpu.VMEM((NSUB, D, QS), _BF16),
    pltpu.VMEM((NSUB, 2, D, FS), _BF16),
    pltpu.VMEM((NSUB, FS + QS, D), _BF16),
    pltpu.VMEM((S // 2, DH), jnp.uint32),
    pltpu.VMEM((NXC, DH // 2, XC), jnp.uint32),
    pltpu.VMEM((NXC, 16, XC), _F32),
    pltpu.VMEM((S, 128), _F32),
    pltpu.VMEM((QR, 2, NG, 64, TQ), jnp.uint32),
    pltpu.VMEM((S, D), _F32),
    pltpu.VMEM((S, D), _BF16),
    pltpu.VMEM((2 * HPS, 48, TQ), _F32),
    pltpu.VMEM((2 * DH + 16, D), _BF16),
    pltpu.VMEM((8, 128), _BF16),
    pltpu.SMEM((2 * HPS,), jnp.int32),
    pltpu.SemaphoreType.DMA((NXC + 3 + 6 + 1,)),
]


@jax.jit
def pallas_gated_mix__grouped_kv_mqa__glu_gated_reglu__prompt_kernel(
    A_x: jax.Array,
    A_wq: jax.Array,
    A_wk: jax.Array,
    A_wv: jax.Array,
    A_wo: jax.Array,
    B_x: jax.Array,
    B_W_gate: jax.Array,
    B_W_up: jax.Array,
    B_W_down: jax.Array,
    gate_w: jax.Array,
):
    del B_x
    any_spec = pl.BlockSpec(memory_space=pl.ANY)
    out = pl.pallas_call(
        _kernel,
        in_specs=[any_spec] * 9,
        out_specs=any_spec,
        out_shape=jax.ShapeDtypeStruct((S, D), _BF16),
        scratch_shapes=_SCRATCH,
        compiler_params=pltpu.CompilerParams(vmem_limit_bytes=100 * 1024 * 1024),
        name="gmix",
    )(A_x.reshape(S, D), A_wq, A_wk.T, A_wv.T, A_wo, B_W_gate, B_W_up, B_W_down,
      gate_w.reshape(8, 128))
    return out.reshape(1, S, D)
```
